```python
import os as _os
_os.environ.setdefault("JAX_PLATFORMS", "cpu")
import jax
import jax.numpy as jnp

def _softmax(x, axis=-1):
    return jax.nn.softmax(x, axis=axis)
def _gelu(x):
    return jax.nn.gelu(x, approximate=True)
def _silu(x):
    return jax.nn.silu(x)
def _sigmoid(x):
    return jax.nn.sigmoid(x)
def _layernorm(x, axis=-1, eps=1e-5):
    m = jnp.mean(x, axis=axis, keepdims=True)
    v = jnp.var(x, axis=axis, keepdims=True)
    return (x - m) / jnp.sqrt(v + eps)
def _scatter_add(tgt, idx, src, axis=0):
    return tgt.at[idx].add(src)
def _segment_sum(src, seg, n):
    return jax.ops.segment_sum(src, seg, n)
class _Rng:
    def __init__(self, key):
        self._k = key
    def _next(self):
        self._k, sub = jax.random.split(self._k)
        return sub
    def normal(self, shape):
        return jax.random.normal(self._next(), shape, dtype=jnp.bfloat16)
    def randint(self, lo, hi, shape):
        return jax.random.randint(self._next(), shape, lo, hi, dtype=jnp.int32)
    def uniform(self, shape, lo=0.0, hi=1.0):
        return jax.random.uniform(self._next(), shape, jnp.bfloat16, lo, hi)
    def permutation(self, n):
        return jax.random.permutation(self._next(), n)


kernel_name = 'concat_heads__mha_block_cached__mha_block_cached__near_ridge'

def setup_inputs():
    _rng = _Rng(jax.random.key(int.from_bytes(__import__("os").urandom(4), "little")))
    _w = (lambda a: (lambda t: t.astype(jnp.bfloat16) if jnp.issubdtype(t.dtype, jnp.floating) else t)(jnp.asarray(a)))
    def _A_setup():
        B, Sq, D = 8, 144, 640
        H, Sk, Dh = 32, 512, 128
        return {
            "x": _w((lambda *s: _rng.normal(s) * 0.8)(B, Sq, D)),
            "k_cache": _w((lambda *s: _rng.normal(s) * 0.8)(B, H, Sk, Dh)),
            "v_cache": _w((lambda *s: _rng.normal(s) * 0.05)(B, H, Sk, Dh)),
            "wq": _w((lambda *s: _rng.normal(s) * 0.8)(D, H * Dh) * (D ** -0.5)),
            "wo": _w((lambda *s: _rng.normal(s) * 0.05)(H * Dh, D) * ((H * Dh) ** -0.5)),
        }
    _A_in = _A_setup()

    def _B_setup():
        B, Sq, D = 8, 144, 640
        H, Sk, Dh = 32, 512, 128
        return {
            "x": _w((lambda *s: _rng.normal(s) * 0.8)(B, Sq, D)),
            "k_cache": _w((lambda *s: _rng.normal(s) * 0.8)(B, H, Sk, Dh)),
            "v_cache": _w((lambda *s: _rng.normal(s) * 0.05)(B, H, Sk, Dh)),
            "wq": _w((lambda *s: _rng.normal(s) * 0.8)(D, H * Dh) * (D ** -0.5)),
            "wo": _w((lambda *s: _rng.normal(s) * 0.05)(H * Dh, D) * ((H * Dh) ** -0.5)),
        }
    _B_in = _B_setup()

    return {
        "A_x": _A_in["x"],
        "A_k_cache": _A_in["k_cache"],
        "A_v_cache": _A_in["v_cache"],
        "A_wq": _A_in["wq"],
        "A_wo": _A_in["wo"],
        "B_x": _B_in["x"],
        "B_k_cache": _B_in["k_cache"],
        "B_v_cache": _B_in["v_cache"],
        "B_wq": _B_in["wq"],
        "B_wo": _B_in["wo"],
    }

def reference(A_x, A_k_cache, A_v_cache, A_wq, A_wo, B_x, B_k_cache, B_v_cache, B_wq, B_wo):
    def _A_ref(x, k_cache, v_cache, wq, wo):
        B, Sq, D = x.shape
        H, Dh = 32, 128
        q = (lambda x, *d: x.transpose(*d))((x @ wq).reshape(B, Sq, H, Dh), 0, 2, 1, 3)
        scores = jnp.einsum("bhqd,bhkd->bhqk", q, k_cache) * (Dh ** -0.5)
        p = _softmax(scores, axis=-1)
        o = jnp.einsum("bhqk,bhkd->bhqd", p, v_cache)
        return (lambda x, *d: x.transpose(*d))(o, 0, 2, 1, 3).reshape(B, Sq, H * Dh) @ wo

    def _B_ref(x, k_cache, v_cache, wq, wo):
        B, Sq, D = x.shape
        H, Dh = 32, 128
        q = (lambda x, *d: x.transpose(*d))((x @ wq).reshape(B, Sq, H, Dh), 0, 2, 1, 3)
        scores = jnp.einsum("bhqd,bhkd->bhqk", q, k_cache) * (Dh ** -0.5)
        p = _softmax(scores, axis=-1)
        o = jnp.einsum("bhqk,bhkd->bhqd", p, v_cache)
        return (lambda x, *d: x.transpose(*d))(o, 0, 2, 1, 3).reshape(B, Sq, H * Dh) @ wo

    a = _A_ref(A_x, A_k_cache, A_v_cache, A_wq, A_wo)
    b = _B_ref(B_x, B_k_cache, B_v_cache, B_wq, B_wo)
    return jnp.concatenate([a, b], axis=-1)
```

```python
import functools
import math
import jax
import jax.numpy as jnp
from jax import lax
import jax.experimental.pallas as pl
import jax.experimental.pallas.tpu as pltpu

B, SQ, D = 8, 144, 640
H, SK, DH = 32, 512, 128
G = 4
HG = H // G
GD = G * DH
T = HG * B
NS = 4
P = NS - 1
WQ_ROWS = D // B
WO_ROWS = GD // B
QSCALE = (DH ** -0.5) * math.log2(math.e)
F32 = jnp.float32
BF16 = jnp.bfloat16


def _kernel(xa_hbm, ka_hbm, va_hbm, wqa_hbm, woa_hbm,
            xb_hbm, kb_hbm, vb_hbm, wqb_hbm, wob_hbm,
            out_hbm,
            xbuf, kbuf, vbuf, wqbuf, wobuf, acc, obuf,
            sem_x, sem_kv, sem_w, sem_o):
    x_hbm = (xa_hbm, xb_hbm)
    k_hbm = (ka_hbm, kb_hbm)
    v_hbm = (va_hbm, vb_hbm)
    wq_hbm = (wqa_hbm, wqb_hbm)
    wo_hbm = (woa_hbm, wob_hbm)

    def x_copy(blk, b):
        return pltpu.make_async_copy(x_hbm[blk].at[b], xbuf.at[blk, b], sem_x.at[blk, b])

    def kv_copy(which, blk, t, slot):
        g = t // B
        b = t % B
        src = (k_hbm, v_hbm)[which][blk]
        dst = (kbuf, vbuf)[which]
        return pltpu.make_async_copy(src.at[b, pl.ds(g * G, G)], dst.at[slot, blk],
                                     sem_kv.at[slot, 2 * blk + which])

    def wq_full(blk, g, slot):
        return pltpu.make_async_copy(wq_hbm[blk].at[:, pl.ds(g * GD, GD)], wqbuf.at[slot, blk],
                                     sem_w.at[slot, blk])

    def wo_full(blk, g, slot):
        return pltpu.make_async_copy(wo_hbm[blk].at[pl.ds(g * GD, GD), :], wobuf.at[slot, blk],
                                     sem_w.at[slot, 2 + blk])

    def wq_piece(blk, g, slot, i):
        r = pl.multiple_of(i * WQ_ROWS, 16)
        return pltpu.make_async_copy(wq_hbm[blk].at[pl.ds(r, WQ_ROWS), pl.ds(g * GD, GD)],
                                     wqbuf.at[slot, blk, pl.ds(r, WQ_ROWS), :], sem_w.at[slot, blk])

    def wo_piece(blk, g, slot, i):
        r = pl.multiple_of(i * WO_ROWS, 16)
        return pltpu.make_async_copy(wo_hbm[blk].at[pl.ds(g * GD + r, WO_ROWS), :],
                                     wobuf.at[slot, blk, pl.ds(r, WO_ROWS), :], sem_w.at[slot, 2 + blk])

    def out_copy(b):
        return pltpu.make_async_copy(obuf.at[b], out_hbm.at[b], sem_o.at[b])

    def start_weight_piece(u):
        gn = jnp.minimum(u // B + 1, HG - 1)
        slot = (u // B + 1) % 2
        i = u % B
        for blk in range(2):
            wq_piece(blk, gn, slot, i).start()
            wo_piece(blk, gn, slot, i).start()

    def start_kv(t):
        tc = jnp.minimum(t, T - 1)
        for blk in range(2):
            kv_copy(0, blk, tc, t % NS).start()
            kv_copy(1, blk, tc, t % NS).start()

    for blk in range(2):
        x_copy(blk, 0).start()
        wq_full(blk, 0, 0).start()
    for blk in range(2):
        kv_copy(0, blk, 0, 0).start()
        kv_copy(1, blk, 0, 0).start()
    for blk in range(2):
        wo_full(blk, 0, 0).start()
    acc[...] = jnp.zeros(acc.shape, F32)
    for blk in range(2):
        x_copy(blk, 0).wait()
        wq_full(blk, 0, 0).wait()
        wo_full(blk, 0, 0).wait()
    for t0 in range(1, P):
        for blk in range(2):
            kv_copy(0, blk, t0, t0).start()
            kv_copy(1, blk, t0, t0).start()
        if t0 == 1:
            for blk in range(2):
                x_copy(blk, 1).start()
    start_weight_piece(0)

    def qproj(blk, b, wslot):
        q = jnp.dot(xbuf[blk, b], wqbuf[wslot, blk], preferred_element_type=F32)
        return [(q[:, h * DH:(h + 1) * DH] * QSCALE).astype(BF16) for h in range(G)]

    def qk(q, blk, slot, h):
        return lax.dot_general(q[h], kbuf[slot, blk, h], (((1,), (1,)), ((), ())),
                               preferred_element_type=F32)

    def softmax(s):
        m = jnp.max(s, axis=-1, keepdims=True)
        p = jnp.exp2(s - m)
        l = jnp.sum(p, axis=-1, keepdims=True)
        return p.astype(BF16), l

    def pv(p, l, blk, slot, h):
        o = jnp.dot(p, vbuf[slot, blk, h], preferred_element_type=F32)
        r = pl.reciprocal(l, approx=True)
        r = r * (2.0 - l * r)
        return (o * r).astype(BF16)

    def oproj(os, blk, wslot):
        return jnp.dot(jnp.concatenate(os, axis=1), wobuf[wslot, blk], preferred_element_type=F32)

    def body(t, carry, run_ahead):
        g = t // B
        b = t % B
        slot = t % NS
        wslot = g % 2

        @pl.when(g == 0)
        def _():
            @pl.when(b + 2 < B)
            def _():
                for blk in range(2):
                    x_copy(blk, b + 2).start()
            @pl.when(b > 0)
            def _():
                for blk in range(2):
                    x_copy(blk, b).wait()

        @pl.when(jnp.logical_and(b == 0, g > 0))
        def _():
            for blk in range(2):
                wq_full(blk, g, wslot).wait()
                wo_full(blk, g, wslot).wait()

        for blk in range(2):
            kv_copy(0, blk, t, slot).wait()
            kv_copy(1, blk, t, slot).wait()

        qa = qproj(0, b, wslot)
        sa = [qk(qa, 0, slot, h) for h in range(G)]
        qb = qproj(1, b, wslot)
        pa = [softmax(s) for s in sa]
        oa = [pv(p, l, 0, slot, h) for h, (p, l) in enumerate(pa)]
        sb = [qk(qb, 1, slot, h) for h in range(G)]
        ya = oproj(oa, 0, wslot)
        pb = [softmax(s) for s in sb]
        acc[b, :, 0:D] += ya
        ob = [pv(p, l, 1, slot, h) for h, (p, l) in enumerate(pb)]
        yb = oproj(ob, 1, wslot)
        if run_ahead:
            start_kv(t + P)
            start_weight_piece(t + 1)
        acc[b, :, D:2 * D] += yb

        @pl.when(g == HG - 1)
        def _():
            obuf[b] = acc[b].astype(BF16)
            out_copy(b).start()
        return carry

    lax.fori_loop(0, T - P, functools.partial(body, run_ahead=True), 0)
    lax.fori_loop(T - P, T, functools.partial(body, run_ahead=False), 0)

    nsur = T - P + 1 - B * (HG - 1)
    for blk in range(2):
        pltpu.make_async_copy(wq_hbm[blk].at[pl.ds(0, nsur * WQ_ROWS), pl.ds(0, GD)],
                              wqbuf.at[HG % 2, blk, pl.ds(0, nsur * WQ_ROWS), :], sem_w.at[HG % 2, blk]).wait()
        pltpu.make_async_copy(wo_hbm[blk].at[pl.ds(0, nsur * WO_ROWS), :],
                              wobuf.at[HG % 2, blk, pl.ds(0, nsur * WO_ROWS), :], sem_w.at[HG % 2, 2 + blk]).wait()
    for b in range(B):
        out_copy(b).wait()


@jax.jit
def pallas_concat_heads__mha_block_cached__mha_block_cached__near_ridge_kernel(
        A_x, A_k_cache, A_v_cache, A_wq, A_wo, B_x, B_k_cache, B_v_cache, B_wq, B_wo):
    any_spec = pl.BlockSpec(memory_space=pl.ANY)
    return pl.pallas_call(
        _kernel,
        in_specs=[any_spec] * 10,
        out_specs=any_spec,
        out_shape=jax.ShapeDtypeStruct((B, SQ, 2 * D), BF16),
        scratch_shapes=[
            pltpu.VMEM((2, B, SQ, D), BF16),
            pltpu.VMEM((NS, 2, G, SK, DH), BF16),
            pltpu.VMEM((NS, 2, G, SK, DH), BF16),
            pltpu.VMEM((2, 2, D, GD), BF16),
            pltpu.VMEM((2, 2, GD, D), BF16),
            pltpu.VMEM((B, SQ, 2 * D), F32),
            pltpu.VMEM((B, SQ, 2 * D), BF16),
            pltpu.SemaphoreType.DMA((2, B)),
            pltpu.SemaphoreType.DMA((NS, 4)),
            pltpu.SemaphoreType.DMA((2, 4)),
            pltpu.SemaphoreType.DMA((B,)),
        ],
        compiler_params=pltpu.CompilerParams(vmem_limit_bytes=100 * 1024 * 1024, disable_bounds_checks=True),
    )(A_x, A_k_cache, A_v_cache, A_wq, A_wo, B_x, B_k_cache, B_v_cache, B_wq, B_wo)
```
